```python
import os as _os
_os.environ.setdefault("JAX_PLATFORMS", "cpu")
import jax
import jax.numpy as jnp

def _softmax(x, axis=-1):
    return jax.nn.softmax(x, axis=axis)
def _gelu(x):
    return jax.nn.gelu(x, approximate=True)
def _silu(x):
    return jax.nn.silu(x)
def _sigmoid(x):
    return jax.nn.sigmoid(x)
def _layernorm(x, axis=-1, eps=1e-5):
    m = jnp.mean(x, axis=axis, keepdims=True)
    v = jnp.var(x, axis=axis, keepdims=True)
    return (x - m) / jnp.sqrt(v + eps)
def _scatter_add(tgt, idx, src, axis=0):
    return tgt.at[idx].add(src)
def _segment_sum(src, seg, n):
    return jax.ops.segment_sum(src, seg, n)
class _Rng:
    def __init__(self, key):
        self._k = key
    def _next(self):
        self._k, sub = jax.random.split(self._k)
        return sub
    def normal(self, shape):
        return jax.random.normal(self._next(), shape, dtype=jnp.bfloat16)
    def randint(self, lo, hi, shape):
        return jax.random.randint(self._next(), shape, lo, hi, dtype=jnp.int32)
    def uniform(self, shape, lo=0.0, hi=1.0):
        return jax.random.uniform(self._next(), shape, jnp.bfloat16, lo, hi)
    def permutation(self, n):
        return jax.random.permutation(self._next(), n)


kernel_name = 'gated_mix__sliding_block__sliding_local_dilated__prompt'

def setup_inputs():
    _rng = _Rng(jax.random.key(int.from_bytes(__import__("os").urandom(4), "little")))
    _w = (lambda a: (lambda t: t.astype(jnp.bfloat16) if jnp.issubdtype(t.dtype, jnp.floating) else t)(jnp.asarray(a)))
    def _A_setup():
        B, S, D = 1, 2048, 640
        return {
            "x": _w((lambda *s: _rng.normal(s) * 0.05)(B, S, D)),
            "wqkv": _w((lambda *s: _rng.normal(s) * 0.8)(D, 3 * D)),
            "wo": _w((lambda *s: _rng.normal(s) * 0.05)(D, D)),
        }
    _A_in = _A_setup()

    def _B_setup():
        B, S, D = 1, 2048, 640
        return {
            "x": _w((lambda *s: _rng.normal(s) * 0.05)(B, S, D)),
            "wqkv": _w((lambda *s: _rng.normal(s) * 0.8)(D, 3 * D)),
            "wo": _w((lambda *s: _rng.normal(s) * 0.05)(D, D)),
        }
    _B_in = _B_setup()

    return {
        "A_x": _A_in["x"],
        "A_wqkv": _A_in["wqkv"],
        "A_wo": _A_in["wo"],
        "B_x": _B_in["x"],
        "B_wqkv": _B_in["wqkv"],
        "B_wo": _B_in["wo"],
        "gate_w": _w((lambda *s: _rng.normal(s) * 0.05)(640) * 16.0),
    }

def reference(A_x, A_wqkv, A_wo, B_x, B_wqkv, B_wo, gate_w):
    def _A_ref(x, wqkv, wo):
        B, S, D = x.shape
        H = 32; Dh = D // H; W = 256
        qkv = (lambda x, *d: x.transpose(*d))((x @ wqkv).reshape(B, S, 3, H, Dh), 2, 0, 3, 1, 4)
        q, k, v = qkv[0], qkv[1], qkv[2]
        scores = jnp.einsum("bhqd,bhkd->bhqk", q, k) * (Dh ** -0.5)
        idx = jnp.arange(S)
        mask = (idx[:, None] - idx[None, :] >= 0) & (idx[:, None] - idx[None, :] < W)
        scores = jnp.where(mask[None, None], scores, -1e9)
        p = _softmax(scores, axis=-1)
        o = jnp.einsum("bhqk,bhkd->bhqd", p, v)
        return (lambda x, *d: x.transpose(*d))(o, 0, 2, 1, 3).reshape(B, S, D) @ wo

    def _B_ref(x, wqkv, wo):
        B, S, D = x.shape
        H = 32; Dh = D // H
        W, dil = 8, 2
        qkv = (lambda x, *d: x.transpose(*d))((x @ wqkv).reshape(B, S, 3, H, Dh), 2, 0, 3, 1, 4)
        q, k, v = qkv[0], qkv[1], qkv[2]
        scale = Dh ** -0.5
        pos = jnp.arange(S)
        off = jnp.arange(W) * dil
        idx = pos[:, None] - off[None, :]
        mask = idx >= 0
        idx_c = jnp.where(mask, idx, 0).reshape(-1)
        kg = k[:, :, idx_c, :].reshape(B, H, S, W, Dh)
        vg = v[:, :, idx_c, :].reshape(B, H, S, W, Dh)
        logits = jnp.einsum("bhsd,bhswd->bhsw", q, kg) * scale
        logits = jnp.where(mask[None, None, :, :], logits, -1e9)
        attn = _softmax(logits, axis=-1)
        o = jnp.einsum("bhsw,bhswd->bhsd", attn, vg)
        return (lambda x, *d: x.transpose(*d))(o, 0, 2, 1, 3).reshape(B, S, D) @ wo

    x = A_x
    g = _sigmoid((x * gate_w).sum(-1, keepdims=True))
    a = _A_ref(x, A_wqkv, A_wo)
    b = _B_ref(x, B_wqkv, B_wo)
    return g * a + (1 - g) * b
```

```python
import functools
import math

import jax
import jax.numpy as jnp
import jax.experimental.pallas as pl
import jax.experimental.pallas.tpu as pltpu

S = 2048
D = 640
H = 32
DH = 20
TM = 256
NB = S // TM
QSCALE = (DH ** -0.5) * math.log2(math.e)
NT_DIMS = (((1,), (1,)), ((), ()))
F32 = jnp.float32
BF16 = jnp.bfloat16
U32 = jnp.uint32
BPAD = 16
RC = 32


def _iota(shape, dim):
    return jax.lax.broadcasted_iota(jnp.int32, shape, dim)


def _kernel(x_hbm, wa_hbm, woa_hbm, wb_hbm, wob_hbm, gw_hbm, out_hbm,
            x_v, wa_v, wb_v, woa_v, wob_v, gw_v, wo_v, wbt_v, tmp_v,
            q_s, k_s, vt_s, g_s, oat_s, kb_s, vb_s, qb_s, ob_s, out_s,
            s0, s1, p0, p1, sems, osems):
    cps = [pltpu.make_async_copy(src, dst, sems.at[i]) for i, (src, dst) in enumerate((
        (x_hbm, x_v), (wa_hbm, wa_v), (wb_hbm, wb_v), (woa_hbm, woa_v), (wob_hbm, wob_v), (gw_hbm, gw_v)))]
    for c in cps:
        c.start()

    lane = _iota((64, 128), 1)
    row = _iota((64, 128), 0)
    tri = row <= (lane & 63)
    lane32 = _iota((32, 128), 1)
    lane48 = _iota((48, 128), 1)
    row48 = _iota((48, 128), 0)
    lane128 = _iota((128, 128), 1)
    ones_rows = jnp.where(_iota((8, TM), 0) == 0, 1.0, 0.0).astype(F32)

    kb_s[:, 0:BPAD, :] = jnp.zeros((5, BPAD, 128), F32)
    vb_s[:, 0:BPAD, :] = jnp.zeros((5, BPAD, 128), F32)
    for buf in (p0, p1):
        buf[...] = jnp.zeros(buf.shape, U32)

    cps[2].wait()
    for t in range(3):
        for nt in range(5):
            blk = wb_v[:, t * D + nt * 128: t * D + (nt + 1) * 128].astype(F32)
            for ft in range(5):
                tmp_v[ft, nt * 128:(nt + 1) * 128, :] = blk[ft * 128:(ft + 1) * 128, :].T
        for ft in range(5):
            for dp in range(10):
                pieces = []
                for d in (2 * dp, 2 * dp + 1):
                    for hq in range(4):
                        pieces.append(tmp_v[ft, pl.ds(hq * 160 + d, 8, stride=20), :])
                wbt_v[t * D + dp * 64: t * D + (dp + 1) * 64, ft * 128:(ft + 1) * 128] = (
                    jnp.concatenate(pieces, axis=0).astype(BF16))
    cps[3].wait()
    cps[4].wait()
    wo_v[0:D, :] = woa_v[...]
    for ft in range(5):
        tmp_v[ft] = wob_v[:, ft * 128:(ft + 1) * 128].astype(F32)
    for ft in range(5):
        for dp in range(10):
            pieces = []
            for d in (2 * dp, 2 * dp + 1):
                for hq in range(4):
                    pieces.append(tmp_v[ft, pl.ds(hq * 160 + d, 8, stride=20), :])
            wo_v[D + dp * 64: D + (dp + 1) * 64, ft * 128:(ft + 1) * 128] = (
                jnp.concatenate(pieces, axis=0).astype(BF16))

    cps[0].wait()
    cps[1].wait()
    cps[5].wait()

    def proj_a(m, c):
        r0 = pl.multiple_of(m * TM, TM)
        w0 = pl.multiple_of(m * (TM // 2), TM // 2)
        xm = x_v[pl.ds(r0, TM), :]
        for src_off, dst, scale in ((0, q_s, QSCALE), (D, k_s, None)):
            r = jnp.dot(xm, wa_v[:, src_off:src_off + D], preferred_element_type=F32)
            if scale is not None:
                r = r * scale
            ru = pltpu.bitcast(r.astype(BF16), U32)
            rolled = []
            for g in range(5):
                rg = ru[:, g * 128:(g + 1) * 128]
                dst[g, pl.ds(w0, TM // 2), :] = rg
                rolled.append(pltpu.roll(rg, 64, 1))
            for i in range(4):
                dst[5 + i, pl.ds(w0, TM // 2), :] = jnp.where(lane128 < 64, rolled[i], rolled[i + 1])
        v = jnp.dot(xm, wa_v[:, 2 * D:3 * D], preferred_element_type=F32)
        vt = v.T
        for p in range(16):
            blk = jnp.concatenate([vt[40 * p:40 * p + 40], ones_rows], axis=0)
            vt_s[p, :, pl.ds(r0, TM)] = pltpu.bitcast(blk.astype(BF16), U32)
        z = jnp.sum(xm.astype(F32) * gw_v[...].astype(F32), axis=1, keepdims=True)
        g_s[pl.ds(r0, TM), :] = jnp.broadcast_to(jax.nn.sigmoid(z), (TM, 128))
        return c

    jax.lax.fori_loop(0, NB, proj_a, 0)

    def proj_b(m):
        r0 = pl.multiple_of(m * TM, TM)
        xm = x_v[pl.ds(r0, TM), :]
        q = jax.lax.dot_general(xm, wbt_v[0:D, :], NT_DIMS, preferred_element_type=F32) * QSCALE
        k = jax.lax.dot_general(xm, wbt_v[D:2 * D, :], NT_DIMS, preferred_element_type=F32)
        v = jax.lax.dot_general(xm, wbt_v[2 * D:3 * D, :], NT_DIMS, preferred_element_type=F32)
        for j in range(5):
            qb_s[j, pl.ds(r0, TM), :] = q[:, j * 128:(j + 1) * 128]
            kb_s[j, pl.ds(r0 + BPAD, TM), :] = k[:, j * 128:(j + 1) * 128]
            vb_s[j, pl.ds(r0 + BPAD, TM), :] = v[:, j * 128:(j + 1) * 128]

    def attn_b(m):
        r0 = pl.multiple_of(m * TM, TM)
        for c in range(TM // RC):
            rc = pl.multiple_of(r0 + c * RC, RC)
            qs = [qb_s[j, pl.ds(rc, RC), :] for j in range(5)]
            ss = []
            for w in range(8):
                acc = None
                for j in range(5):
                    t = qs[j] * kb_s[j, pl.ds(rc + (BPAD - 2 * w), RC), :]
                    acc = t if acc is None else acc + t
                acc = acc + pltpu.roll(acc, 64, 1)
                acc = acc + pltpu.roll(acc, 32, 1)
                if c == 0 and w > 0:
                    pos = rc + _iota((RC, 128), 0)
                    acc = jnp.where(pos >= 2 * w, acc, -1e9)
                ss.append(acc)
            mx = functools.reduce(jnp.maximum, ss)
            es = [jnp.exp2(s - mx) for s in ss]
            l = functools.reduce(lambda a, b: a + b, es)
            sc = (1.0 - g_s[pl.ds(rc, RC), :]) / l
            for j in range(5):
                acc = None
                for w in range(8):
                    t = es[w] * vb_s[j, pl.ds(rc + (BPAD - 2 * w), RC), :]
                    acc = t if acc is None else acc + t
                ob_s[pl.ds(rc, RC), j * 128:(j + 1) * 128] = (acc * sc).astype(BF16)

    proj_b(0)

    def phase2(m, c):
        proj_b(m)
        attn_b(m - 1)
        return c

    jax.lax.fori_loop(1, NB, phase2, 0)
    attn_b(NB - 1)

    def pair_idx(p):
        f0 = p * 40
        g0 = f0 >> 7
        o0 = f0 & 127
        strad = o0 + 40 > 128
        g = jnp.where(strad, 5 + ((f0 - 64) >> 7), g0)
        o = jnp.where(strad, (f0 - 64) & 127, o0)
        return g, o

    def make_stages(first):
        def split(it):
            if first:
                return it, 0
            return it & 15, (1 + (it >> 4)) * TM

        def stage_a(it, sb):
            p, qb = split(it)
            g, o = pair_idx(p)
            m0 = (lane32 >= o) & (lane32 < o + DH)
            m1 = (lane32 >= o + DH) & (lane32 < o + 2 * DH)
            for j in range(4):
                q = q_s[g, pl.ds(pl.multiple_of(qb // 2 + j * 32, 32), 32), :]
                qm = jnp.concatenate([jnp.where(m0, q, 0), jnp.where(m1, q, 0)], axis=0)
                qm = pltpu.bitcast(qm, BF16)
                if first:
                    nk = 64 * (j + 1)
                    k = pltpu.bitcast(k_s[g, 0:nk // 2, :], BF16)
                    sb[j, 320 - nk:320, :] = jax.lax.dot_general(k, qm, NT_DIMS, preferred_element_type=F32)
                else:
                    k = pltpu.bitcast(k_s[g, pl.ds(pl.multiple_of(qb // 2 - 128 + j * 32, 32), 160), :], BF16)
                    sb[j] = jax.lax.dot_general(k, qm, NT_DIMS, preferred_element_type=F32)

        def stage_b(it, sb, pb):
            for j in range(4):
                off = 0 if j % 2 == 0 else 32
                if first:
                    bot = jnp.where(tri, sb[j, 256:320, :], -1e30)
                    if j > 0:
                        mid = sb[j, 256 - 64 * j:256, :]
                        m = jnp.maximum(jnp.max(bot, axis=0, keepdims=True), jnp.max(mid, axis=0, keepdims=True))
                        pmid = jnp.exp2(mid - m)
                        pb[j, off + 128 - 32 * j:off + 128, :] = pltpu.bitcast(pmid.astype(BF16), U32)
                    else:
                        m = jnp.max(bot, axis=0, keepdims=True)
                    pb[j, off + 128:off + 160, :] = pltpu.bitcast(jnp.exp2(bot - m).astype(BF16), U32)
                else:
                    sm = jnp.where(tri, sb[j, 256:320, :], sb[j, 0:64, :])
                    mid = sb[j, 64:256, :]
                    m = jnp.maximum(jnp.max(sm, axis=0, keepdims=True), jnp.max(mid, axis=0, keepdims=True))
                    pm = jnp.exp2(sm - m)
                    pmid = jnp.exp2(mid - m)
                    pb[j, off:off + 32, :] = pltpu.bitcast(jnp.where(tri, 0.0, pm).astype(BF16), U32)
                    pb[j, off + 32:off + 128, :] = pltpu.bitcast(pmid.astype(BF16), U32)
                    pb[j, off + 128:off + 160, :] = pltpu.bitcast(jnp.where(tri, pm, 0.0).astype(BF16), U32)

        def stage_c(it, pb):
            p, qb = split(it)
            res = []
            for j in range(4):
                if first:
                    nkt = 1 if j < 2 else 2
                    hi = 160 if j % 2 == 0 else 192
                    lo = hi + (32 if j % 2 == 0 else 0) - 64 * nkt
                    hi = lo + 64 * nkt
                    pt = pltpu.bitcast(pb[j, lo:hi, :], BF16)
                    vt = pltpu.bitcast(vt_s[p, :, 0:128 * nkt], BF16)
                else:
                    k0 = qb - 256 + (j // 2) * 128
                    vt = pltpu.bitcast(vt_s[p, :, pl.ds(pl.multiple_of(k0, 128), 384)], BF16)
                    pt = pltpu.bitcast(pb[j], BF16)
                ot = jnp.dot(vt, pt, preferred_element_type=F32)
                res.append(ot * (1.0 / ot[40:41]))
            for j in range(2):
                a, b = res[2 * j], res[2 * j + 1]
                z = jnp.where(row48 < DH, b, a)
                w = jnp.where(row48 < DH, a, b)
                out = jnp.where((lane48 < 64) == (row48 < DH), w, pltpu.roll(z, 64, 1))
                oat_s[pl.ds(pl.multiple_of(p * 40, 8), 40), pl.ds(pl.multiple_of(qb + j * 128, 128), 128)] = out[0:40]

        return stage_a, stage_b, stage_c

    def run_pipeline(first, n):
        sa, sb_, sc = make_stages(first)
        sa(0, s0)
        sb_(0, s0, p0)
        sa(1, s1)

        def body(i2, c):
            it = 2 + 2 * i2
            sc(it - 2, p0)
            sa(it, s0)
            sb_(it - 1, s1, p1)
            sc(it - 1, p1)
            sa(it + 1, s1)
            sb_(it, s0, p0)
            return c

        jax.lax.fori_loop(0, (n - 2) // 2, body, 0)
        sc(n - 2, p0)
        sb_(n - 1, s1, p1)
        sc(n - 1, p1)

    run_pipeline(True, 16)
    for buf in (p0, p1):
        buf[...] = jnp.zeros(buf.shape, U32)
    run_pipeline(False, 16 * (NB - 1))

    def out_copy(m):
        r = pl.ds(pl.multiple_of(m * TM, TM), TM)
        return pltpu.make_async_copy(out_s.at[r, :], out_hbm.at[r, :], osems.at[m])

    def proj_o(m, c):
        r0 = pl.multiple_of(m * TM, TM)
        oa = oat_s[:, pl.ds(r0, TM)].T * jnp.concatenate([g_s[pl.ds(r0, TM), :]] * 5, axis=1)
        lhs = jnp.concatenate([oa.astype(BF16), ob_s[pl.ds(r0, TM), :]], axis=1)
        out_s[pl.ds(r0, TM), :] = jnp.dot(lhs, wo_v[...], preferred_element_type=F32).astype(BF16)
        out_copy(m).start()
        return c

    jax.lax.fori_loop(0, NB, proj_o, 0)
    for m in range(NB):
        out_copy(m).wait()


@jax.jit
def pallas_gated_mix__sliding_block__sliding_local_dilated__prompt_kernel(
    A_x: jax.Array,
    A_wqkv: jax.Array,
    A_wo: jax.Array,
    B_x: jax.Array,
    B_wqkv: jax.Array,
    B_wo: jax.Array,
    gate_w: jax.Array,
):
    del B_x
    x = A_x.reshape(S, D)
    gw = gate_w.reshape(1, D)
    V = pltpu.VMEM
    scratch = [
        V((S, D), BF16), V((D, 3 * D), BF16), V((D, 3 * D), BF16), V((D, D), BF16), V((D, D), BF16),
        V((1, D), BF16), V((2 * D, D), BF16), V((3 * D, D), BF16), V((5, D, 128), F32),
        V((9, S // 2, 128), U32), V((9, S // 2, 128), U32), V((16, 24, S), U32),
        V((S, 128), F32), V((D, S), F32),
        V((5, S + BPAD, 128), F32), V((5, S + BPAD, 128), F32), V((5, S, 128), F32),
        V((S, D), BF16), V((S, D), BF16),
        V((4, 320, 128), F32), V((4, 320, 128), F32), V((4, 192, 128), U32), V((4, 192, 128), U32),
        pltpu.SemaphoreType.DMA((6,)), pltpu.SemaphoreType.DMA((NB,)),
    ]
    out = pl.pallas_call(
        _kernel,
        out_shape=jax.ShapeDtypeStruct((S, D), BF16),
        in_specs=[pl.BlockSpec(memory_space=pl.ANY)] * 6,
        out_specs=pl.BlockSpec(memory_space=pl.ANY),
        scratch_shapes=scratch,
        compiler_params=pltpu.CompilerParams(vmem_limit_bytes=110 * 1024 * 1024),
    )(x, A_wqkv, A_wo, B_wqkv, B_wo, gw)
    return out.reshape(1, S, D)
```

```python
import functools
import math

import jax
import jax.numpy as jnp
import jax.experimental.pallas as pl
import jax.experimental.pallas.tpu as pltpu

S = 2048
D = 640
H = 32
DH = 20
TM = 256
NB = S // TM
QSCALE = (DH ** -0.5) * math.log2(math.e)
NT_DIMS = (((1,), (1,)), ((), ()))
F32 = jnp.float32
BF16 = jnp.bfloat16
U32 = jnp.uint32
BPAD = 16
ORDER = 'C0 C1 C2 C3 A0 A1 A2 A3 B0 B1 B2 B3'
UNR = 5
BCH = 64
OPOS = 2
FLAGS = {}
PU = 2
RC = 32


def _iota(shape, dim):
    return jax.lax.broadcasted_iota(jnp.int32, shape, dim)


def _kernel(x_hbm, wa_hbm, woa_hbm, wb_hbm, wob_hbm, gw_hbm, out_hbm,
            x_v, wa_v, wb_v, woa_v, wob_v, gw_v, wo_v, wbt_v, tmp_v,
            q_b, k_b, vt_b, g_s, oat_s, kb_s, vb_s, qb_s, ob_s, out_s,
            s0, s1, p0, p1, sems, osems):
    cps = [pltpu.make_async_copy(src, dst, sems.at[i]) for i, (src, dst) in enumerate((
        (x_hbm.at[0:TM, :], x_v.at[0:TM, :]), (wa_hbm, wa_v), (wb_hbm, wb_v), (woa_hbm, woa_v), (wob_hbm, wob_v), (gw_hbm, gw_v)))]
    for i in (0, 1, 5):
        cps[i].start()

    q_s, k_s, vt_s = q_b.bitcast(U32), k_b.bitcast(U32), vt_b.bitcast(U32)
    lane = _iota((64, 128), 1)
    row = _iota((64, 128), 0)
    tri = row <= (lane & 63)
    lane32 = _iota((32, 128), 1)
    lane48 = _iota((48, 128), 1)
    row48 = _iota((48, 128), 0)
    lane128 = _iota((128, 128), 1)
    ones_rows = jnp.where(_iota((8, TM), 0) == 0, 1.0, 0.0).astype(F32)

    kb_s[:, 0:BPAD, :] = jnp.zeros((5, BPAD, 128), F32)
    vb_s[:, 0:BPAD, :] = jnp.zeros((5, BPAD, 128), F32)
    for buf in (p0, p1):
        buf[...] = jnp.zeros(buf.shape, BF16)

    cps[0].wait()
    cps[1].wait()
    cps[5].wait()

    def x_copy(m):
        r = pl.ds(pl.multiple_of(m * TM, TM), TM)
        return pltpu.make_async_copy(x_hbm.at[r, :], x_v.at[r, :], osems.at[m])

    for m in range(1, NB):
        x_copy(m).start()
    for i in (2, 3, 4):
        cps[i].start()

    def proj_a(m, c, prep=False):
        r0 = pl.multiple_of(m * TM, TM)
        w0 = pl.multiple_of(m * (TM // 2), TM // 2)

        if prep:
            for u in range(3):
                n0 = pl.multiple_of(((m - 3) * 3 + u) * 128, 128)
                for ft in range(5):
                    tmp_v[ft, pl.ds(n0, 128), :] = wb_v[ft * 128:(ft + 1) * 128, pl.ds(n0, 128)].astype(F32).T

        xm = x_v[pl.ds(r0, TM), :]
        for src_off, dst, scale in ((0, q_b, QSCALE), (D, k_b, None)):
            r = jnp.dot(xm, wa_v[:, src_off:src_off + D], preferred_element_type=F32)
            if scale is not None:
                r = r * scale
            for g in range(5):
                dst[g, pl.ds(r0, TM), :] = r[:, g * 128:(g + 1) * 128].astype(BF16)
            dst = dst.bitcast(U32)
            rolled = [pltpu.roll(dst[g, pl.ds(w0, TM // 2), :], 64, 1) for g in range(5)]
            for i in range(4):
                dst[5 + i, pl.ds(w0, TM // 2), :] = jnp.where(lane128 < 64, rolled[i], rolled[i + 1])
        v = jnp.dot(xm, wa_v[:, 2 * D:3 * D], preferred_element_type=F32)
        vt = v.T
        for p in range(16):
            blk = jnp.concatenate([vt[40 * p:40 * p + 40], ones_rows], axis=0)
            vt_b[p, :, pl.ds(r0, TM)] = blk.astype(BF16)
        z = jnp.sum(xm.astype(F32) * gw_v[...].astype(F32), axis=1, keepdims=True)
        g_s[pl.ds(r0, TM), :] = jnp.broadcast_to(jax.nn.sigmoid(z), (TM, 128))
        return c

    proj_a(0, 0)
    for m in range(1, NB):
        x_copy(m).wait()
    jax.lax.fori_loop(1, 3, proj_a, 0)
    cps[2].wait()
    jax.lax.fori_loop(3, NB, functools.partial(proj_a, prep=True), 0)

    for t in range(3):
        for ft in range(5):
            for dp in range(10):
                pieces = []
                for d in (2 * dp, 2 * dp + 1):
                    for hq in range(4):
                        pieces.append(tmp_v[ft, pl.ds(t * D + hq * 160 + d, 8, stride=20), :])
                wbt_v[t * D + dp * 64: t * D + (dp + 1) * 64, ft * 128:(ft + 1) * 128] = (
                    jnp.concatenate(pieces, axis=0).astype(BF16))
    cps[3].wait()
    cps[4].wait()
    wo_v[0:D, :] = woa_v[...]
    for ft in range(5):
        tmp_v[ft, 0:D, :] = wob_v[:, ft * 128:(ft + 1) * 128].astype(F32)
    for ft in range(5):
        for dp in range(10):
            pieces = []
            for d in (2 * dp, 2 * dp + 1):
                for hq in range(4):
                    pieces.append(tmp_v[ft, pl.ds(hq * 160 + d, 8, stride=20), :])
            wo_v[D + dp * 64: D + (dp + 1) * 64, ft * 128:(ft + 1) * 128] = (
                jnp.concatenate(pieces, axis=0).astype(BF16))

    def proj_b(m):
        r0 = pl.multiple_of(m * TM, TM)
        xm = x_v[pl.ds(r0, TM), :]
        q = jax.lax.dot_general(xm, wbt_v[0:D, :], NT_DIMS, preferred_element_type=F32) * QSCALE
        k = jax.lax.dot_general(xm, wbt_v[D:2 * D, :], NT_DIMS, preferred_element_type=F32)
        v = jax.lax.dot_general(xm, wbt_v[2 * D:3 * D, :], NT_DIMS, preferred_element_type=F32)
        for j in range(5):
            qb_s[j, pl.ds(r0, TM), :] = q[:, j * 128:(j + 1) * 128]
            kb_s[j, pl.ds(r0 + BPAD, TM), :] = k[:, j * 128:(j + 1) * 128]
            vb_s[j, pl.ds(r0 + BPAD, TM), :] = v[:, j * 128:(j + 1) * 128]

    def attn_b(rc, masked):
        if True:
            rc = pl.multiple_of(rc, RC)
            qs = [qb_s[j, pl.ds(rc, RC), :] for j in range(5)]
            ss = []
            for w in range(8):
                acc = None
                for j in range(5):
                    t = qs[j] * kb_s[j, pl.ds(rc + (BPAD - 2 * w), RC), :]
                    acc = t if acc is None else acc + t
                acc = acc + pltpu.roll(acc, 64, 1)
                acc = acc + pltpu.roll(acc, 32, 1)
                if masked and w > 0:
                    pos = rc + _iota((RC, 128), 0)
                    acc = jnp.where(pos >= 2 * w, acc, -1e9)
                ss.append(acc)
            mx = functools.reduce(jnp.maximum, ss)
            es = [jnp.exp2(s - mx) for s in ss]
            l = functools.reduce(lambda a, b: a + b, es)
            sc = (1.0 - g_s[pl.ds(rc, RC), :]) / l
            for j in range(5):
                acc = None
                for w in range(8):
                    t = es[w] * vb_s[j, pl.ds(rc + (BPAD - 2 * w), RC), :]
                    acc = t if acc is None else acc + t
                ob_s[pl.ds(rc, RC), j * 128:(j + 1) * 128] = (acc * sc).astype(BF16)

    def phase2(m, c):
        proj_b(m)
        return c

    jax.lax.fori_loop(0, NB, phase2, 0, unroll=PU)

    def pair_idx(p):
        f0 = p * 40
        g0 = f0 >> 7
        o0 = f0 & 127
        strad = o0 + 40 > 128
        g = jnp.where(strad, 5 + ((f0 - 64) >> 7), g0)
        o = jnp.where(strad, (f0 - 64) & 127, o0)
        return g, o

    def make_stages(first):
        def split(it):
            if first:
                return it, 0
            return it & 15, jnp.where(it < 0, S, (1 + (it >> 4)) * TM)

        def stage_a(it, sb, j):
            p, qb = split(it)
            g, o = pair_idx(p)
            m0 = (lane32 >= o) & (lane32 < o + DH)
            m1 = (lane32 >= o + DH) & (lane32 < o + 2 * DH)
            q = q_s[g, pl.ds(pl.multiple_of(qb // 2 + j * 32, 32), 32), :]
            qm = jnp.concatenate([jnp.where(m0, q, 0), jnp.where(m1, q, 0)], axis=0)
            qm = pltpu.bitcast(qm, BF16)
            if first:
                nk = 64 * (j + 1)
                k = pltpu.bitcast(k_s[g, 0:nk // 2, :], BF16)
                s = jax.lax.dot_general(k, qm, NT_DIMS, preferred_element_type=F32)
                sm = jnp.where(tri, s[nk - 64:nk], -1e30)
                m = jnp.max(sm, axis=0, keepdims=True)
                if j > 0:
                    m = jnp.maximum(m, jnp.max(s[0:nk - 64], axis=0, keepdims=True))
                    sb[j, 256 - (nk - 64):256, :] = s[0:nk - 64]
            else:
                k = pltpu.bitcast(k_s[g, pl.ds(pl.multiple_of(qb // 2 - 128 + j * 32, 32), 160), :], BF16)
                s = jax.lax.dot_general(k, qm, NT_DIMS, preferred_element_type=F32)
                sm = jnp.where(tri, s[256:320], s[0:64])
                m = jnp.maximum(jnp.max(sm, axis=0, keepdims=True), jnp.max(s[64:256], axis=0, keepdims=True))
                sb[j, 64:256, :] = s[64:256]
            sb[j, 0:64, :] = sm
            sb[j, 256:264, :] = jnp.broadcast_to(m, (8, 128))

        def stage_b(sb, pb, j):
            off = 0 if j % 2 == 0 else 64
            m = sb[j, 256:257, :]
            pm = jnp.exp2(sb[j, 0:64, :] - m)
            if first:
                if j > 0:
                    pb[j, off + 256 - 64 * j:off + 256, :] = jnp.exp2(sb[j, 256 - 64 * j:256, :] - m).astype(BF16)
                pb[j, off + 256:off + 320, :] = pm.astype(BF16)
            else:
                pb[j, off:off + 64, :] = jnp.where(tri, 0.0, pm).astype(BF16)
                pb[j, off + 256:off + 320, :] = jnp.where(tri, pm, 0.0).astype(BF16)
                for r in range(64, 256, BCH):
                    pb[j, off + r:off + r + BCH, :] = jnp.exp2(sb[j, r:r + BCH, :] - m).astype(BF16)

        res = {}

        def stage_c(it, pb, j):
            p, qb = split(it)
            pb = pb.bitcast(U32)
            if first:
                nkt = 1 if j < 2 else 2
                pt = pltpu.bitcast(pb[j, 192 - 64 * nkt:192, :], BF16)
                vt = pltpu.bitcast(vt_s[p, :, 0:128 * nkt], BF16)
            else:
                k0 = qb - 256 + (j // 2) * 128
                vt = pltpu.bitcast(vt_s[p, :, pl.ds(pl.multiple_of(k0, 128), 384)], BF16)
                pt = pltpu.bitcast(pb[j], BF16)
            ot = jnp.dot(vt, pt, preferred_element_type=F32)
            res[j] = ot * (1.0 / ot[40:41])
            if j % 2 == 1:
                a, b = res[j - 1], res[j]
                z = jnp.where(row48 < DH, b, a)
                w = jnp.where(row48 < DH, a, b)
                out = jnp.where((lane48 < 64) == (row48 < DH), w, pltpu.roll(z, 64, 1))
                oat_s[pl.ds(pl.multiple_of(p * 40, 8), 40),
                      pl.ds(pl.multiple_of(qb + (j // 2) * 128, 128), 128)] = out[0:40]

        def half(ia, sa, sb, pb, ic, pc):
            for tok in ORDER.split():
                j = int(tok[1])
                if tok[0] == "A" and ia is not None:
                    stage_a(ia, sa, j)
                elif tok[0] == "B" and sb is not None:
                    stage_b(sb, pb, j)
                elif tok[0] == "C" and ic is not None:
                    stage_c(ic, pc, j)

        return half

    def out_copy(m):
        r = pl.ds(m * TM, TM)
        return pltpu.make_async_copy(out_s.at[r, :], out_hbm.at[r, :], osems.at[m])

    def proj_o(m):
        r0 = pl.multiple_of(m * TM, TM)
        oa = oat_s[:, pl.ds(r0, TM)].T * jnp.concatenate([g_s[pl.ds(r0, TM), :]] * 5, axis=1)
        lhs = jnp.concatenate([oa.astype(BF16), ob_s[pl.ds(r0, TM), :]], axis=1)
        out_s[pl.ds(r0, TM), :] = jnp.dot(lhs, wo_v[...], preferred_element_type=F32).astype(BF16)

    half = make_stages(True)
    half(0, s0, None, None, None, None)
    half(1, s1, s0, p0, None, None)

    def body0(i2, c):
        half(2 + 2 * i2, s0, s1, p1, 2 * i2, p0)
        half(3 + 2 * i2, s1, s0, p0, 2 * i2 + 1, p1)
        attn_b(i2 * RC, True)
        return c

    jax.lax.fori_loop(0, 7, body0, 0)
    attn_b(7 * RC, True)
    half(None, None, s1, p1, 14, p0)
    half(None, None, None, None, 15, p1)

    for buf in (s0, s1, p0, p1):
        buf[...] = jnp.zeros(buf.shape, buf.dtype)
    half = make_stages(False)

    def body1(i, c):
        for h in range(0, 16, 2):
            it = 16 * i + h
            half(it, s0, s1, p1, it - 2, p0)
            half(it + 1, s1, s0, p0, it - 1, p1)
            attn_b((i + 1) * TM + (h // 2) * RC, False)
            if h == OPOS:
                proj_o(i)
        r = pl.ds(pl.multiple_of(i * TM, TM), TM)
        pltpu.make_async_copy(out_s.at[r, :], out_hbm.at[r, :], osems.at[i]).start()
        return c

    jax.lax.fori_loop(0, NB - 1, body1, 0)
    n = 16 * (NB - 1)
    half(None, None, s1, p1, n - 2, p0)
    half(None, None, None, None, n - 1, p1)
    proj_o(NB - 1)
    out_copy(NB - 1).start()
    for m in range(NB):
        out_copy(m).wait()


@jax.jit
def pallas_gated_mix__sliding_block__sliding_local_dilated__prompt_kernel(
    A_x: jax.Array,
    A_wqkv: jax.Array,
    A_wo: jax.Array,
    B_x: jax.Array,
    B_wqkv: jax.Array,
    B_wo: jax.Array,
    gate_w: jax.Array,
):
    del B_x
    x = A_x.reshape(S, D)
    gw = gate_w.reshape(1, D)
    V = pltpu.VMEM
    scratch = [
        V((S, D), BF16), V((D, 3 * D), BF16), V((D, 3 * D), BF16), V((D, D), BF16), V((D, D), BF16),
        V((1, D), BF16), V((2 * D, D), BF16), V((3 * D, D), BF16), V((5, 3 * D, 128), F32),
        V((9, S, 128), BF16), V((9, S, 128), BF16), V((16, 48, S + TM), BF16),
        V((S, 128), F32), V((D, S + TM), F32),
        V((5, S + BPAD, 128), F32), V((5, S + BPAD, 128), F32), V((5, S, 128), F32),
        V((S, D), BF16), V((S, D), BF16),
        V((4, 264, 128), F32), V((4, 264, 128), F32), V((4, 384, 128), BF16), V((4, 384, 128), BF16),
        pltpu.SemaphoreType.DMA((6,)), pltpu.SemaphoreType.DMA((NB,)),
    ]
    out = pl.pallas_call(
        _kernel,
        out_shape=jax.ShapeDtypeStruct((S, D), BF16),
        in_specs=[pl.BlockSpec(memory_space=pl.ANY)] * 6,
        out_specs=pl.BlockSpec(memory_space=pl.ANY),
        scratch_shapes=scratch,
        compiler_params=pltpu.CompilerParams(vmem_limit_bytes=110 * 1024 * 1024, flags=FLAGS or None),
    )(x, A_wqkv, A_wo, B_wqkv, B_wo, gw)
    return out.reshape(1, S, D)
```

```python
import functools
import math

import jax
import jax.numpy as jnp
import jax.experimental.pallas as pl
import jax.experimental.pallas.tpu as pltpu

S = 2048
D = 640
H = 32
DH = 20
TM = 256
NB = S // TM
QSCALE = (DH ** -0.5) * math.log2(math.e)
NT_DIMS = (((1,), (1,)), ((), ()))
F32 = jnp.float32
BF16 = jnp.bfloat16
U32 = jnp.uint32
BPAD = 16
ORDER = 'C0 C1 C2 C3 A0 A1 A2 A3 B0 B1 B2 B3'
UNR = 5
BCH = 64
OPOS = 2
FLAGS = {}
PU = 2
FUSE = 1
HB = 8
PPOS = 0
RC = 16


def _iota(shape, dim):
    return jax.lax.broadcasted_iota(jnp.int32, shape, dim)


def _kernel(x_hbm, wa_hbm, woa_hbm, wb_hbm, wob_hbm, gw_hbm, out_hbm,
            x_v, wa_v, wb_v, woa_v, wob_v, gw_v, wo_v, wbt_v, tmp_v,
            q_b, k_b, vt_b, g_s, oat_s, kb_s, vb_s, qb_s, ob_s, out_s,
            s0, s1, p0, p1, sems, osems):
    cps = [pltpu.make_async_copy(src, dst, sems.at[i]) for i, (src, dst) in enumerate((
        (x_hbm.at[0:TM, :], x_v.at[0:TM, :]), (wa_hbm, wa_v), (wb_hbm, wb_v), (woa_hbm, woa_v), (wob_hbm, wob_v), (gw_hbm, gw_v)))]
    for i in (0, 1, 5):
        cps[i].start()

    q_s, k_s, vt_s = q_b.bitcast(U32), k_b.bitcast(U32), vt_b.bitcast(U32)
    lane = _iota((64, 128), 1)
    row = _iota((64, 128), 0)
    tri = row <= (lane & 63)
    lane32 = _iota((32, 128), 1)
    lane48 = _iota((48, 128), 1)
    row48 = _iota((48, 128), 0)
    lane128 = _iota((128, 128), 1)
    ones_rows = jnp.where(_iota((8, TM), 0) == 0, 1.0, 0.0).astype(F32)

    kb_s[:, 0:BPAD, :] = jnp.zeros((5, BPAD, 128), F32)
    vb_s[:, 0:BPAD, :] = jnp.zeros((5, BPAD, 128), F32)
    for buf in (p0, p1):
        buf[...] = jnp.zeros(buf.shape, BF16)

    cps[0].wait()
    cps[1].wait()
    cps[5].wait()

    def x_copy(m):
        r = pl.ds(pl.multiple_of(m * TM, TM), TM)
        return pltpu.make_async_copy(x_hbm.at[r, :], x_v.at[r, :], osems.at[m])

    for m in range(1, NB):
        x_copy(m).start()
    for i in (2, 3, 4):
        cps[i].start()

    def proj_a(m, c, prep=False):
        r0 = pl.multiple_of(m * TM, TM)
        w0 = pl.multiple_of(m * (TM // 2), TM // 2)

        if prep:
            for u in range(3):
                n0 = pl.multiple_of(((m - 3) * 3 + u) * 128, 128)
                for ft in range(5):
                    tmp_v[ft, pl.ds(n0, 128), :] = wb_v[ft * 128:(ft + 1) * 128, pl.ds(n0, 128)].astype(F32).T

        xm = x_v[pl.ds(r0, TM), :]
        for src_off, dst, scale in ((0, q_b, QSCALE), (D, k_b, None)):
            r = jnp.dot(xm, wa_v[:, src_off:src_off + D], preferred_element_type=F32)
            if scale is not None:
                r = r * scale
            for g in range(5):
                dst[g, pl.ds(r0, TM), :] = r[:, g * 128:(g + 1) * 128].astype(BF16)
            dst = dst.bitcast(U32)
            rolled = [pltpu.roll(dst[g, pl.ds(w0, TM // 2), :], 64, 1) for g in range(5)]
            for i in range(4):
                dst[5 + i, pl.ds(w0, TM // 2), :] = jnp.where(lane128 < 64, rolled[i], rolled[i + 1])
        v = jnp.dot(xm, wa_v[:, 2 * D:3 * D], preferred_element_type=F32)
        vt = v.T
        for p in range(16):
            blk = jnp.concatenate([vt[40 * p:40 * p + 40], ones_rows], axis=0)
            vt_b[p, :, pl.ds(r0, TM)] = blk.astype(BF16)
        z = jnp.sum(xm.astype(F32) * gw_v[...].astype(F32), axis=1, keepdims=True)
        g_s[pl.ds(r0, TM), :] = jnp.broadcast_to(jax.nn.sigmoid(z), (TM, 128))
        return c

    proj_a(0, 0)
    for m in range(1, NB):
        x_copy(m).wait()
    jax.lax.fori_loop(1, 3, proj_a, 0)
    cps[2].wait()
    jax.lax.fori_loop(3, NB, functools.partial(proj_a, prep=True), 0)

    for t in range(3):
        for ft in range(5):
            for dp in range(10):
                pieces = []
                for d in (2 * dp, 2 * dp + 1):
                    for hq in range(4):
                        pieces.append(tmp_v[ft, pl.ds(t * D + hq * 160 + d, 8, stride=20), :])
                wbt_v[t * D + dp * 64: t * D + (dp + 1) * 64, ft * 128:(ft + 1) * 128] = (
                    jnp.concatenate(pieces, axis=0).astype(BF16))
    cps[3].wait()
    cps[4].wait()
    wo_v[0:D, :] = woa_v[...]
    for ft in range(5):
        tmp_v[ft, 0:D, :] = wob_v[:, ft * 128:(ft + 1) * 128].astype(F32)
    for ft in range(5):
        for dp in range(10):
            pieces = []
            for d in (2 * dp, 2 * dp + 1):
                for hq in range(4):
                    pieces.append(tmp_v[ft, pl.ds(hq * 160 + d, 8, stride=20), :])
            wo_v[D + dp * 64: D + (dp + 1) * 64, ft * 128:(ft + 1) * 128] = (
                jnp.concatenate(pieces, axis=0).astype(BF16))

    def proj_b(m):
        r0 = pl.multiple_of(m * TM, TM)
        xm = x_v[pl.ds(r0, TM), :]
        q = jax.lax.dot_general(xm, wbt_v[0:D, :], NT_DIMS, preferred_element_type=F32) * QSCALE
        k = jax.lax.dot_general(xm, wbt_v[D:2 * D, :], NT_DIMS, preferred_element_type=F32)
        v = jax.lax.dot_general(xm, wbt_v[2 * D:3 * D, :], NT_DIMS, preferred_element_type=F32)
        for j in range(5):
            qb_s[j, pl.ds(r0, TM), :] = q[:, j * 128:(j + 1) * 128]
            kb_s[j, pl.ds(r0 + BPAD, TM), :] = k[:, j * 128:(j + 1) * 128]
            vb_s[j, pl.ds(r0 + BPAD, TM), :] = v[:, j * 128:(j + 1) * 128]

    def attn_b(rc, masked):
        rbase = rc
        for cc in range(32 // RC):
            rc = pl.multiple_of(rbase + cc * RC, RC)
            qs = [qb_s[j, pl.ds(rc, RC), :] for j in range(5)]
            ss = []
            for w in range(8):
                acc = None
                for j in range(5):
                    t = qs[j] * kb_s[j, pl.ds(rc + (BPAD - 2 * w), RC), :]
                    acc = t if acc is None else acc + t
                acc = acc + pltpu.roll(acc, 64, 1)
                acc = acc + pltpu.roll(acc, 32, 1)
                if masked and w > 0:
                    pos = rc + _iota((RC, 128), 0)
                    acc = jnp.where(pos >= 2 * w, acc, -1e9)
                ss.append(acc)
            mx = functools.reduce(jnp.maximum, ss)
            es = [jnp.exp2(s - mx) for s in ss]
            l = functools.reduce(lambda a, b: a + b, es)
            sc = (1.0 - g_s[pl.ds(rc, RC), :]) / l
            for j in range(5):
                acc = None
                for w in range(8):
                    t = es[w] * vb_s[j, pl.ds(rc + (BPAD - 2 * w), RC), :]
                    acc = t if acc is None else acc + t
                ob_s[pl.ds(rc, RC), j * 128:(j + 1) * 128] = (acc * sc).astype(BF16)

    def phase2(m, c):
        proj_b(m)
        return c

    if FUSE:
        proj_b(0)
    else:
        jax.lax.fori_loop(0, NB, phase2, 0, unroll=PU)

    def pair_idx(p):
        f0 = p * 40
        g0 = f0 >> 7
        o0 = f0 & 127
        strad = o0 + 40 > 128
        g = jnp.where(strad, 5 + ((f0 - 64) >> 7), g0)
        o = jnp.where(strad, (f0 - 64) & 127, o0)
        return g, o

    def make_stages(first):
        def split(it):
            if first:
                return it, 0
            return it & 15, jnp.where(it < 0, S, (1 + (it >> 4)) * TM)

        def stage_a(it, sb, j):
            p, qb = split(it)
            g, o = pair_idx(p)
            m0 = (lane32 >= o) & (lane32 < o + DH)
            m1 = (lane32 >= o + DH) & (lane32 < o + 2 * DH)
            q = q_s[g, pl.ds(pl.multiple_of(qb // 2 + j * 32, 32), 32), :]
            qm = jnp.concatenate([jnp.where(m0, q, 0), jnp.where(m1, q, 0)], axis=0)
            qm = pltpu.bitcast(qm, BF16)
            if first:
                nk = 64 * (j + 1)
                k = pltpu.bitcast(k_s[g, 0:nk // 2, :], BF16)
                s = jax.lax.dot_general(k, qm, NT_DIMS, preferred_element_type=F32)
                sm = jnp.where(tri, s[nk - 64:nk], -1e30)
                m = jnp.max(sm, axis=0, keepdims=True)
                if j > 0:
                    m = jnp.maximum(m, jnp.max(s[0:nk - 64], axis=0, keepdims=True))
                    sb[j, 256 - (nk - 64):256, :] = s[0:nk - 64]
            else:
                k = pltpu.bitcast(k_s[g, pl.ds(pl.multiple_of(qb // 2 - 128 + j * 32, 32), 160), :], BF16)
                s = jax.lax.dot_general(k, qm, NT_DIMS, preferred_element_type=F32)
                sm = jnp.where(tri, s[256:320], s[0:64])
                m = jnp.maximum(jnp.max(sm, axis=0, keepdims=True), jnp.max(s[64:256], axis=0, keepdims=True))
                sb[j, 64:256, :] = s[64:256]
            sb[j, 0:64, :] = sm
            sb[j, 256:264, :] = jnp.broadcast_to(m, (8, 128))

        def stage_b(sb, pb, j):
            off = 0 if j % 2 == 0 else 64
            m = sb[j, 256:257, :]
            pm = jnp.exp2(sb[j, 0:64, :] - m)
            if first:
                if j > 0:
                    pb[j, off + 256 - 64 * j:off + 256, :] = jnp.exp2(sb[j, 256 - 64 * j:256, :] - m).astype(BF16)
                pb[j, off + 256:off + 320, :] = pm.astype(BF16)
            else:
                pb[j, off:off + 64, :] = jnp.where(tri, 0.0, pm).astype(BF16)
                pb[j, off + 256:off + 320, :] = jnp.where(tri, pm, 0.0).astype(BF16)
                for r in range(64, 256, BCH):
                    pb[j, off + r:off + r + BCH, :] = jnp.exp2(sb[j, r:r + BCH, :] - m).astype(BF16)

        res = {}

        def stage_c(it, pb, j):
            p, qb = split(it)
            pb = pb.bitcast(U32)
            if first:
                nkt = 1 if j < 2 else 2
                pt = pltpu.bitcast(pb[j, 192 - 64 * nkt:192, :], BF16)
                vt = pltpu.bitcast(vt_s[p, :, 0:128 * nkt], BF16)
            else:
                k0 = qb - 256 + (j // 2) * 128
                vt = pltpu.bitcast(vt_s[p, :, pl.ds(pl.multiple_of(k0, 128), 384)], BF16)
                pt = pltpu.bitcast(pb[j], BF16)
            ot = jnp.dot(vt, pt, preferred_element_type=F32)
            res[j] = ot * (1.0 / ot[40:41])
            if j % 2 == 1:
                a, b = res[j - 1], res[j]
                z = jnp.where(row48 < DH, b, a)
                w = jnp.where(row48 < DH, a, b)
                out = jnp.where((lane48 < 64) == (row48 < DH), w, pltpu.roll(z, 64, 1))
                oat_s[pl.ds(pl.multiple_of(p * 40, 8), 40),
                      pl.ds(pl.multiple_of(qb + (j // 2) * 128, 128), 128)] = out[0:40]

        def half(ia, sa, sb, pb, ic, pc):
            for tok in ORDER.split():
                j = int(tok[1])
                if tok[0] == "A" and ia is not None:
                    stage_a(ia, sa, j)
                elif tok[0] == "B" and sb is not None:
                    stage_b(sb, pb, j)
                elif tok[0] == "C" and ic is not None:
                    stage_c(ic, pc, j)

        return half

    def out_copy(m):
        r = pl.ds(m * TM, TM)
        return pltpu.make_async_copy(out_s.at[r, :], out_hbm.at[r, :], osems.at[m])

    def proj_o(m):
        r0 = pl.multiple_of(m * TM, TM)
        oa = oat_s[:, pl.ds(r0, TM)].T * jnp.concatenate([g_s[pl.ds(r0, TM), :]] * 5, axis=1)
        lhs = jnp.concatenate([oa.astype(BF16), ob_s[pl.ds(r0, TM), :]], axis=1)
        out_s[pl.ds(r0, TM), :] = jnp.dot(lhs, wo_v[...], preferred_element_type=F32).astype(BF16)

    half = make_stages(True)
    half(0, s0, None, None, None, None)
    half(1, s1, s0, p0, None, None)

    def body0(i2, c):
        half(2 + 2 * i2, s0, s1, p1, 2 * i2, p0)
        half(3 + 2 * i2, s1, s0, p0, 2 * i2 + 1, p1)
        attn_b(i2 * 32, True)
        return c

    jax.lax.fori_loop(0, 7, body0, 0)
    attn_b(7 * 32, True)
    half(None, None, s1, p1, 14, p0)
    half(None, None, None, None, 15, p1)

    for buf in (s0, s1, p0, p1):
        buf[...] = jnp.zeros(buf.shape, buf.dtype)
    half = make_stages(False)

    def body1(i, c):
        for h in range(0, 16, 2):
            it = 16 * i + h
            half(it, s0, s1, p1, it - 2, p0)
            half(it + 1, s1, s0, p0, it - 1, p1)
            if h >= HB:
                n = 16 // (16 - HB)
                for u in range(n):
                    attn_b((i + 1) * TM + ((h - HB) // 2 * n + u) * 32, False)
            if h == PPOS:
                proj_b(i + 1)
            if h == OPOS:
                proj_o(i)
        r = pl.ds(pl.multiple_of(i * TM, TM), TM)
        pltpu.make_async_copy(out_s.at[r, :], out_hbm.at[r, :], osems.at[i]).start()
        return c

    jax.lax.fori_loop(0, NB - 1, body1, 0)
    n = 16 * (NB - 1)
    half(None, None, s1, p1, n - 2, p0)
    half(None, None, None, None, n - 1, p1)
    proj_o(NB - 1)
    out_copy(NB - 1).start()
    for m in range(NB):
        out_copy(m).wait()


@jax.jit
def pallas_gated_mix__sliding_block__sliding_local_dilated__prompt_kernel(
    A_x: jax.Array,
    A_wqkv: jax.Array,
    A_wo: jax.Array,
    B_x: jax.Array,
    B_wqkv: jax.Array,
    B_wo: jax.Array,
    gate_w: jax.Array,
):
    del B_x
    x = A_x.reshape(S, D)
    gw = gate_w.reshape(1, D)
    V = pltpu.VMEM
    scratch = [
        V((S, D), BF16), V((D, 3 * D), BF16), V((D, 3 * D), BF16), V((D, D), BF16), V((D, D), BF16),
        V((1, D), BF16), V((2 * D, D), BF16), V((3 * D, D), BF16), V((5, 3 * D, 128), F32),
        V((9, S, 128), BF16), V((9, S, 128), BF16), V((16, 48, S + TM), BF16),
        V((S, 128), F32), V((D, S + TM), F32),
        V((5, S + BPAD, 128), F32), V((5, S + BPAD, 128), F32), V((5, S, 128), F32),
        V((S, D), BF16), V((S, D), BF16),
        V((4, 264, 128), F32), V((4, 264, 128), F32), V((4, 384, 128), BF16), V((4, 384, 128), BF16),
        pltpu.SemaphoreType.DMA((6,)), pltpu.SemaphoreType.DMA((NB,)),
    ]
    out = pl.pallas_call(
        _kernel,
        out_shape=jax.ShapeDtypeStruct((S, D), BF16),
        in_specs=[pl.BlockSpec(memory_space=pl.ANY)] * 6,
        out_specs=pl.BlockSpec(memory_space=pl.ANY),
        scratch_shapes=scratch,
        compiler_params=pltpu.CompilerParams(vmem_limit_bytes=110 * 1024 * 1024, flags=FLAGS or None),
    )(x, A_wqkv, A_wo, B_wqkv, B_wo, gw)
    return out.reshape(1, S, D)
```
